```python
import jax
import jax.numpy as jnp

def _softmax(x, axis=-1):
    return jax.nn.softmax(x, axis=axis)
def _gelu(x):
    return jax.nn.gelu(x, approximate=True)
def _silu(x):
    return jax.nn.silu(x)
def _sigmoid(x):
    return jax.nn.sigmoid(x)
def _layernorm(x, axis=-1, eps=1e-5):
    m = jnp.mean(x, axis=axis, keepdims=True)
    v = jnp.var(x, axis=axis, keepdims=True)
    return (x - m) / jnp.sqrt(v + eps)
def _scatter_add(tgt, idx, src, axis=0):
    return tgt.at[idx].add(src)
def _segment_sum(src, seg, n):
    return jax.ops.segment_sum(src, seg, n)
class _Rng:
    def __init__(self, key):
        self._k = key
    def _next(self):
        self._k, sub = jax.random.split(self._k)
        return sub
    def normal(self, shape):
        return jax.random.normal(self._next(), shape, dtype=jnp.bfloat16)
    def randint(self, lo, hi, shape):
        return jax.random.randint(self._next(), shape, lo, hi, dtype=jnp.int32)
    def uniform(self, shape, lo=0.0, hi=1.0):
        return jax.random.uniform(self._next(), shape, jnp.bfloat16, lo, hi)
    def permutation(self, n):
        return jax.random.permutation(self._next(), n)


kernel_name = 'standalone__groupnorm__prompt'

def setup_inputs():
    _rng = _Rng(jax.random.key(int.from_bytes(__import__("os").urandom(4), "little")))
    _w = (lambda a: (lambda t: t.astype(jnp.bfloat16) if jnp.issubdtype(t.dtype, jnp.floating) else t)(jnp.asarray(a)))
    B = 2
    G = 32
    cpg = max(1, 1024 // G)
    C = G * cpg
    H, W = 32, 2048
    return {
        "x": _w((lambda *s: _rng.normal(s) * 0.05)(B, C, H, W)),
        "g": _w((lambda *s: _rng.normal(s) * 0.05)(C) + 1.0),
        "b": _w((lambda *s: _rng.normal(s) * 0.05)(C)),
    }

def reference(x, g, b):
    G = 32
    B, C, H, W = x.shape[0], x.shape[1], x.shape[2], x.shape[3]
    xr = x.reshape(B, G, C // G, H, W)
    mu = xr.mean(axis=(2, 3, 4), keepdims=True)
    var = ((xr - mu) ** 2).mean(axis=(2, 3, 4), keepdims=True)
    xn = (xr - mu) / jnp.sqrt(var + 1e-5)
    xn = xn.reshape(B, C, H, W)
    return xn * g[None, :, None, None] + b[None, :, None, None]
```

```python
import functools

import jax
import jax.numpy as jnp
import jax.experimental.pallas as pl
import jax.experimental.pallas.tpu as pltpu

_G = 32
_EPS = 1e-5


def _gn_kernel(g_ref, b_ref, x_ref, o_ref, *, cpg, h, w):
    gi = pl.program_id(0) % _G
    n = cpg * h * w

    def sum_body(c, acc):
        xc = x_ref[0, c].astype(jnp.float32)
        return acc + xc

    s = jax.lax.fori_loop(0, cpg, sum_body, jnp.zeros((h, w), jnp.float32))
    mean = jnp.sum(s) * (1.0 / n)

    def var_body(c, acc):
        d = x_ref[0, c].astype(jnp.float32) - mean
        return acc + d * d

    v = jax.lax.fori_loop(0, cpg, var_body, jnp.zeros((h, w), jnp.float32))
    var = jnp.sum(v) * (1.0 / n)
    rstd = jax.lax.rsqrt(jnp.full((1, 1), var + _EPS, jnp.float32))

    def norm_body(c, carry):
        ch = gi * cpg + c
        scale = rstd * g_ref[ch]
        xc = x_ref[0, c].astype(jnp.float32)
        o_ref[0, c] = ((xc - mean) * scale + b_ref[ch]).astype(o_ref.dtype)
        return carry

    jax.lax.fori_loop(0, cpg, norm_body, 0)


@jax.jit
def pallas_standalone__groupnorm__prompt_kernel(x, g, b):
    B, C, H, W = x.shape
    cpg = C // _G
    xr = x.reshape(B * _G, cpg, H, W)
    out = pl.pallas_call(
        functools.partial(_gn_kernel, cpg=cpg, h=H, w=W),
        grid=(B * _G,),
        in_specs=[
            pl.BlockSpec(memory_space=pltpu.SMEM),
            pl.BlockSpec(memory_space=pltpu.SMEM),
            pl.BlockSpec((1, cpg, H, W), lambda i: (i, 0, 0, 0)),
        ],
        out_specs=pl.BlockSpec((1, cpg, H, W), lambda i: (i, 0, 0, 0)),
        out_shape=jax.ShapeDtypeStruct(xr.shape, x.dtype),
        compiler_params=pltpu.CompilerParams(
            dimension_semantics=("arbitrary",),
            vmem_limit_bytes=64 * 1024 * 1024,
        ),
    )(g.astype(jnp.float32), b.astype(jnp.float32), xr)
    return out.reshape(B, C, H, W)
```

```python
import functools
import jax
import jax.numpy as jnp
import jax.experimental.pallas as pl
import jax.experimental.pallas.tpu as pltpu

_G = 32
_EPS = 1e-5


def _gn_kernel(x_hbm, g_hbm, b_hbm, o_hbm,
               pool, gb_vmem, gbf_vmem, gb_smem, stat_smem, rsem, wsem, psem,
               *, rounds, spg, rgs, w, cps, dr, dw, r2w_lead, w2r_lead, unroll, do_compute):
    OCT = 8
    rpc = rgs // cps
    slabs_per_batch = _G * spg
    n_slab = rgs * 8 * w
    half = w // 2

    def rd(gslab, lslab, slot):
        return pltpu.make_async_copy(x_hbm.at[gslab], pool.at[lslab], rsem.at[slot])

    def wr(base, k):
        o = k // rgs
        j = k % rgs
        return pltpu.make_async_copy(pool.at[pl.ds(o * OCT, OCT), j],
                                     o_hbm.at[pl.ds(base + o * OCT, OCT), j],
                                     wsem.at[k % dw])

    def slab_stats(ls):
        def p1(j, acc):
            v = pool[ls, j].astype(jnp.float32)
            return acc + (v[:, :half] + v[:, half:])
        acc = jax.lax.fori_loop(0, rgs, p1, jnp.zeros((8, half), jnp.float32), unroll=unroll)
        m = jnp.sum(acc) * (1.0 / n_slab)
        def p2(j, acc):
            d = pool[ls, j].astype(jnp.float32) - m
            dd = d * d
            return acc + (dd[:, :half] + dd[:, half:])
        acc2 = jax.lax.fori_loop(0, rgs, p2, jnp.zeros((8, half), jnp.float32), unroll=unroll)
        return m, jnp.sum(acc2)

    def normalize(base, k):
        o = k // rgs
        j = k % rgs
        for s in range(OCT):
            ls = o * OCT + s
            lg = ls // spg
            mean = stat_smem[0, lg]
            rstd = stat_smem[1, lg]
            c = ((base + ls) % slabs_per_batch) * cps + j // rpc
            scale = rstd * gb_smem[c // 128, c % 128]
            bias = gb_smem[8 + c // 128, c % 128]
            v = pool[ls, j].astype(jnp.float32)
            pool[ls, j] = ((v - mean) * scale + bias).astype(pool.dtype)

    rd(0, 0, 0).start()
    gcp = pltpu.make_async_copy(g_hbm, gb_vmem.at[0], psem.at[0])
    bcp = pltpu.make_async_copy(b_hbm, gb_vmem.at[1], psem.at[1])
    gcp.start(); bcp.start()
    for i in range(1, dr):
        rd(i, i, i).start()
    gcp.wait(); bcp.wait()
    gbf_vmem[0:8, :] = gb_vmem[0].astype(jnp.float32)
    gbf_vmem[8:16, :] = gb_vmem[1].astype(jnp.float32)
    scp = pltpu.make_async_copy(gbf_vmem, gb_smem, psem.at[2])
    scp.start(); scp.wait()

    base = 0
    for r, K in enumerate(rounds):
        S = K * spg
        NW = S // OCT * rgs
        last_round = r == len(rounds) - 1

        def group_body(lg, carry, base=base, S=S, K=K):
            ms, m2s = [], []
            for s in range(spg):
                ls = lg * spg + s
                rd(base + ls, ls, ls % dr).wait()
                @pl.when(ls + dr < S)
                def _():
                    rd(base + ls + dr, ls + dr, ls % dr).start()
                if s == spg - 1 - r2w_lead:
                    @pl.when(lg == K - 1)
                    def _():
                        for k in range(dw):
                            wr(base, k).start()
                if do_compute:
                    m, m2 = slab_stats(ls)
                    ms.append(m); m2s.append(m2)
                if do_compute and s < spg - 1 - r2w_lead:
                    npre = dw + 1
                    nst = spg - 1 - r2w_lead
                    lo = s * npre // nst
                    hi = (s + 1) * npre // nst
                    @pl.when(lg == K - 1)
                    def _():
                        def nb(k, c):
                            normalize(base, k)
                            return c
                        jax.lax.fori_loop(lo, hi, nb, 0)
            if do_compute:
                mean = sum(ms) * (1.0 / spg)
                m2 = sum(m2s) + n_slab * sum((m - mean) * (m - mean) for m in ms)
                var = m2 * (1.0 / (n_slab * spg))
                rstd = jax.lax.rsqrt(jnp.full((8, 128), var + _EPS, jnp.float32))
                stat_smem[0, lg] = mean
                stat_smem[1, lg] = rstd[0, 0]
            return carry

        jax.lax.fori_loop(0, K, group_body, 0)

        def write_body(k, carry, base=base, NW=NW, S=S, last_round=last_round):
            wr(base, k).wait()
            @pl.when(k + dw < NW)
            def _():
                wr(base, k + dw).start()
            if not last_round:
                @pl.when(k == NW - 1 - w2r_lead)
                def _():
                    for i in range(dr):
                        rd(base + S + i, i, i).start()
            if do_compute:
                @pl.when(k + dw + 1 < NW)
                def _():
                    normalize(base, k + dw + 1)
            return carry

        jax.lax.fori_loop(0, NW, write_body, 0)
        base += S


def make(rounds=(16, 16, 16, 16), dr=3, dw=8, r2w_lead=1, w2r_lead=1, unroll=4, do_compute=True, vmem_mb=100):
    @jax.jit
    def f(x, g, b):
        B, C, H, W = x.shape
        cpg = C // _G
        spg = 4
        cps = cpg // spg
        rgs = cps * H // 8
        NS = B * _G * spg
        assert sum(rounds) == B * _G
        xr = x.reshape(NS, rgs, 8, W)
        kmax = max(rounds)
        out = pl.pallas_call(
            functools.partial(_gn_kernel, rounds=rounds, spg=spg, rgs=rgs, w=W, cps=cps, dr=dr, dw=dw,
                              r2w_lead=r2w_lead, w2r_lead=w2r_lead, unroll=unroll, do_compute=do_compute),
            in_specs=[pl.BlockSpec(memory_space=pl.ANY)] * 3,
            out_specs=pl.BlockSpec(memory_space=pl.ANY),
            out_shape=jax.ShapeDtypeStruct(xr.shape, x.dtype),
            scratch_shapes=[
                pltpu.VMEM((kmax * spg, rgs, 8, W), x.dtype),
                pltpu.VMEM((2, 8, 128), g.dtype),
                pltpu.VMEM((16, 128), jnp.float32),
                pltpu.SMEM((16, 128), jnp.float32),
                pltpu.SMEM((2, kmax), jnp.float32),
                pltpu.SemaphoreType.DMA((dr,)),
                pltpu.SemaphoreType.DMA((dw,)),
                pltpu.SemaphoreType.DMA((3,)),
            ],
            compiler_params=pltpu.CompilerParams(vmem_limit_bytes=vmem_mb * 1024 * 1024),
        )(xr, g.reshape(8, 128), b.reshape(8, 128))
        return out.reshape(B, C, H, W)
    return f


_impl = make()


@jax.jit
def pallas_standalone__groupnorm__prompt_kernel(x, g, b):
    return _impl(x, g, b)
```

```python
import functools
import jax
import jax.numpy as jnp
from jax import lax
import jax.experimental.pallas as pl
import jax.experimental.pallas.tpu as pltpu

_G = 32
_EPS = 1e-5
_SPG = 4
_OCT = 2 * _SPG
_NRSEM = 32
_NWSEM = 16


def _log2(n):
    l = n.bit_length() - 1
    assert 1 << l == n, n
    return l


def _shr(x, n):
    if isinstance(x, int):
        return x >> n
    return lax.shift_right_logical(x, jnp.int32(n))


def _gn_kernel(x_hbm, g_hbm, b_hbm, o_hbm,
               pool, gb_vmem, gbf_vmem, gb_smem, stat_smem, rsem, wsem, psem,
               *, n_rounds, n_full, n_last, rgs, w, cps, dr, dw, r2w_lead, w2r_lead, sched, nhi, do_compute,
               wprio):
    rpc = rgs // cps
    lrgs, lrpc = _log2(rgs), _log2(rpc)
    oct_per_batch = _G // 2
    ch_per_oct = _OCT * cps
    n_group = _SPG * rgs * 8 * w
    aw = w // 4
    f32 = jnp.float32

    def rd_start(bo, p, q):
        o = _shr(p, lrgs)
        j = p & (rgs - 1)
        ls = o * _OCT + q * _SPG
        gs = bo * _OCT + ls
        sem = rsem.at[(2 * p + q) & (_NRSEM - 1)]
        if nhi:
            pltpu.make_async_copy(x_hbm.at[pl.ds(gs, nhi), j], pool.at[pl.ds(ls, nhi), j], sem).start(priority=0)
        pltpu.make_async_copy(x_hbm.at[pl.ds(gs + nhi, _SPG - nhi), j],
                              pool.at[pl.ds(ls + nhi, _SPG - nhi), j], sem).start(priority=1)

    def rd_wait(o, j, q):
        v = pool.at[pl.ds(o * _OCT + q * _SPG, _SPG), j]
        p = o * rgs + j
        pltpu.make_async_copy(v, v, rsem.at[(2 * p + q) & (_NRSEM - 1)]).wait()

    def wr(bo, k):
        o = _shr(k, lrgs)
        j = k & (rgs - 1)
        return pltpu.make_async_copy(pool.at[pl.ds(o * _OCT, _OCT), j],
                                     o_hbm.at[pl.ds((bo + o) * _OCT, _OCT), j],
                                     wsem.at[k & (_NWSEM - 1)])

    def fold(v):
        return (v[:, 0 * aw:1 * aw] + v[:, 1 * aw:2 * aw]) + (v[:, 2 * aw:3 * aw] + v[:, 3 * aw:4 * aw])

    def pass1(lg, j, acc):
        for s in range(_SPG):
            acc = acc + fold(pool[lg * _SPG + s, j].astype(f32))
        return acc

    def pass2(lg, j, mean, acc):
        for s in range(_SPG):
            d = pool[lg * _SPG + s, j].astype(f32) - mean
            acc = acc + fold(d * d)
        return acc

    def fin_mean(lg, acc):
        stat_smem[2 * lg] = jnp.sum(acc) * (1.0 / n_group)

    def fin_rstd(lg, acc):
        var = jnp.sum(jnp.sum(acc, axis=1, keepdims=True), axis=0, keepdims=True) * (1.0 / n_group)
        stat_smem[2 * lg + 1] = lax.rsqrt(var + _EPS)[0, 0]

    def normalize(bo, o, j):
        c0 = ((bo + o) & (oct_per_batch - 1)) * ch_per_oct
        row = _shr(c0, 7)
        col0 = (c0 & 127) + _shr(j, lrpc)
        for q in range(2):
            mean = stat_smem[4 * o + 2 * q]
            rstd = stat_smem[4 * o + 2 * q + 1]
            for s in range(q * _SPG, (q + 1) * _SPG):
                scale = rstd * gb_smem[row, col0 + s * cps]
                bias = gb_smem[8 + row, col0 + s * cps]
                v = pool[o * _OCT + s, j].astype(f32)
                pool[o * _OCT + s, j] = ((v - mean) * scale + bias).astype(pool.dtype)

    zeros = lambda: jnp.zeros((8, aw), f32)

    rd_start(0, 0, 0)
    gcp = pltpu.make_async_copy(g_hbm, gb_vmem.at[0], psem.at[0])
    bcp = pltpu.make_async_copy(b_hbm, gb_vmem.at[1], psem.at[1])
    gcp.start(); bcp.start()
    for t in range(1, 2 * dr):
        rd_start(0, t // 2, t % 2)
    gcp.wait(); bcp.wait()
    gbf_vmem[0:8, :] = gb_vmem[0].astype(f32)
    gbf_vmem[8:16, :] = gb_vmem[1].astype(f32)
    scp = pltpu.make_async_copy(gbf_vmem, gb_smem, psem.at[2])
    scp.start()

    def round_body(r, carry):
        bo = r * n_full
        n = jnp.where(r == n_rounds - 1, n_last, n_full) if n_last != n_full else n_full
        NW = n * rgs

        def read_octet(o, po, with_p2, last):
            if with_p2:
                ms = (stat_smem[4 * po], stat_smem[4 * po + 2])
            def step(j, accs, issue, start_writes_after=None):
                accs = list(accs)
                for q in range(2):
                    rd_wait(o, j, q)
                    if issue:
                        rd_start(bo, o * rgs + j + dr, q)
                    if start_writes_after == q:
                        for k in range(dw):
                            wr(bo, k).start(priority=wprio)
                    if do_compute:
                        accs[q] = pass1(2 * o + q, j, accs[q])
                        if with_p2:
                            accs[2 + q] = pass2(2 * po + q, j, ms[q], accs[2 + q])
                return tuple(accs)
            def body(j, accs):
                accs = step(j, accs, True)
                if last and do_compute:
                    @pl.when(j < dw)
                    def _():
                        normalize(bo, 0, j)
                return accs
            accs = tuple(zeros() for _ in range(4 if with_p2 else 2))
            accs = lax.fori_loop(0, rgs - dr if last else rgs, body, accs)
            if last:
                tsw = 2 * rgs - 1 - r2w_lead
                for j in range(rgs - dr, rgs):
                    accs = step(j, accs, False, (tsw - 2 * j) if tsw // 2 == j else None)
            if do_compute:
                fin_mean(2 * o, accs[0]); fin_mean(2 * o + 1, accs[1])
                if with_p2:
                    fin_rstd(2 * po, accs[2]); fin_rstd(2 * po + 1, accs[3])

        def write_octet(o, po, with_p2, j_start):
            if with_p2:
                ms = (stat_smem[4 * po], stat_smem[4 * po + 2])
            def body(j, accs):
                k = o * rgs + j
                if do_compute:
                    normalize(bo, o, j)
                wr(bo, k - dw).wait()
                wr(bo, k).start(priority=wprio)
                if with_p2 and do_compute:
                    accs = (pass2(2 * po, j, ms[0], accs[0]), pass2(2 * po + 1, j, ms[1], accs[1]))
                return accs
            accs = lax.fori_loop(j_start, rgs, body, tuple(zeros() for _ in range(2 if with_p2 else 0)))
            if with_p2 and do_compute:
                fin_rstd(2 * po, accs[0]); fin_rstd(2 * po + 1, accs[1])

        def rloop(o, c):
            if sched == 'R':
                has, po = o >= 1, o - 1
            else:
                has, po = jnp.logical_and(o >= 1, o <= 2), o - 1
            @pl.when(has)
            def _():
                read_octet(o, po, True, False)
            @pl.when(jnp.logical_not(has))
            def _():
                read_octet(o, po, False, False)
            return c
        lax.fori_loop(0, n - 1, rloop, 0)
        @pl.when(r == 0)
        def _():
            scp.wait()
        read_octet(n - 1, n - 2, sched == 'R', True)

        def wloop(o, c):
            if sched == 'R':
                has, po = o == 1, n - 1
            else:
                has, po = jnp.logical_and(o >= 1, o <= n - 2), o + 1
            @pl.when(has)
            def _():
                write_octet(o, po, True, 0)
            @pl.when(jnp.logical_not(has))
            def _():
                write_octet(o, po, False, jnp.where(o == 0, dw, 0))
            return c
        lax.fori_loop(0, n, wloop, 0)

        for i in range(dw):
            wr(bo, NW - dw + i).wait()
            if i == dw - 1 - w2r_lead:
                @pl.when(r < n_rounds - 1)
                def _():
                    for t in range(2 * dr):
                        rd_start(bo + n_full, t // 2, t % 2)
        return carry

    lax.fori_loop(0, n_rounds, round_body, 0)


def make(n_full=8, dr=5, dw=6, r2w_lead=2, w2r_lead=1, sched='W', nhi=1, do_compute=True, vmem_mb=100,
         nobc=False, wprio=0):
    @jax.jit
    def f(x, g, b):
        B, C, H, W = x.shape
        cpg = C // _G
        cps = cpg // _SPG
        rgs = cps * H // 8
        NS = B * _G * _SPG
        n_oct = NS // _OCT
        n_rounds = -(-n_oct // n_full)
        n_last = n_oct - (n_rounds - 1) * n_full
        assert n_last >= 4 and 2 * dr <= _NRSEM and dw <= _NWSEM and r2w_lead < 2 * dr and w2r_lead < dw
        xr = x.reshape(NS, rgs, 8, W)
        out = pl.pallas_call(
            functools.partial(_gn_kernel, n_rounds=n_rounds, n_full=n_full, n_last=n_last, rgs=rgs, w=W, cps=cps,
                              dr=dr, dw=dw, r2w_lead=r2w_lead, w2r_lead=w2r_lead, sched=sched, nhi=nhi,
                              do_compute=do_compute, wprio=wprio),
            in_specs=[pl.BlockSpec(memory_space=pl.ANY)] * 3,
            out_specs=pl.BlockSpec(memory_space=pl.ANY),
            out_shape=jax.ShapeDtypeStruct(xr.shape, x.dtype),
            scratch_shapes=[
                pltpu.VMEM((n_full * _OCT, rgs, 8, W), x.dtype),
                pltpu.VMEM((2, 8, 128), g.dtype),
                pltpu.VMEM((16, 128), jnp.float32),
                pltpu.SMEM((16, 128), jnp.float32),
                pltpu.SMEM((4 * n_full,), jnp.float32),
                pltpu.SemaphoreType.DMA((_NRSEM,)),
                pltpu.SemaphoreType.DMA((_NWSEM,)),
                pltpu.SemaphoreType.DMA((3,)),
            ],
            compiler_params=pltpu.CompilerParams(vmem_limit_bytes=vmem_mb * 1024 * 1024,
                                                 disable_bounds_checks=nobc),
        )(xr, g.reshape(8, 128), b.reshape(8, 128))
        return out.reshape(B, C, H, W)
    return f


_impl = make(n_full=11)


@jax.jit
def pallas_standalone__groupnorm__prompt_kernel(x, g, b):
    return _impl(x, g, b)
```

```python
import functools
import jax
import jax.numpy as jnp
from jax import lax
import jax.experimental.pallas as pl
import jax.experimental.pallas.tpu as pltpu

_G = 32
_EPS = 1e-5
_SPG = 4
_OCT = 2 * _SPG
_BT = 16
_NRSEM = 32
_NWSEM = 16


def _log2(n):
    l = n.bit_length() - 1
    assert 1 << l == n, n
    return l


def _shr(x, n):
    if isinstance(x, int):
        return x >> n
    return lax.shift_right_logical(x, jnp.int32(n))


def _gn_kernel(x_hbm, g_hbm, b_hbm, o_hbm,
               pool, gb_vmem, gbf_vmem, gb_smem, stat_smem, rsem, wsem, psem,
               *, n_rounds, n_full, n_last, tps, cps, rw, sh, dr, dw, r2w_lead, w2r_lead, wsplit, do_compute):
    nb = tps // _BT
    bpc = nb // cps
    lnb, lbpc = _log2(nb), _log2(bpc)
    oct_per_batch = _G // 2
    ch_per_oct = _OCT * cps
    n_group = _SPG * tps * 8 * 128
    spu = rw * _SPG
    f32 = jnp.float32
    AW = 2

    def rd_copy(gs, ls, ns, t0, nt, sem):
        return pltpu.make_async_copy(x_hbm.at[pl.ds(gs, ns), pl.ds(t0, nt)],
                                     pool.at[pl.ds(ls, ns), pl.ds(t0, nt)], sem)

    def rd_start(bs, p, q):
        u = _shr(p, lnb)
        j = p & (nb - 1)
        ls = u * spu + q * _SPG
        gs = bs + ls
        sem = rsem.at[(p * rw + q) & (_NRSEM - 1)]
        def normal():
            t0 = j * _BT - sh
            rd_copy(gs, ls, 1, t0, _BT, sem).start(priority=0)
            rd_copy(gs + 1, ls + 1, _SPG - 1, t0, _BT, sem).start(priority=1)
        def head():
            rd_copy(gs, ls, 1, 0, _BT - sh, sem).start(priority=0)
            rd_copy(gs, ls, _SPG, tps - sh, sh, sem).start(priority=1)
            rd_copy(gs + 1, ls + 1, _SPG - 1, 0, _BT - sh, sem).start(priority=1)
        if sh == 0:
            normal()
        elif isinstance(j, int):
            head() if j == 0 else normal()
        else:
            pl.when(j == 0)(head)
            pl.when(j != 0)(normal)

    def rd_wait(p, q):
        v = pool.at[pl.ds(0, _SPG), pl.ds(0, _BT)]
        pltpu.make_async_copy(v, v, rsem.at[(p * rw + q) & (_NRSEM - 1)]).wait()

    def wr_start(bs, k):
        o = _shr(k, lnb)
        j = k & (nb - 1)
        ht = _BT // wsplit
        for h in range(wsplit):
            pltpu.make_async_copy(pool.at[pl.ds(o * _OCT, _OCT), pl.ds(j * _BT + h * ht, ht)],
                                  o_hbm.at[pl.ds(bs + o * _OCT, _OCT), pl.ds(j * _BT + h * ht, ht)],
                                  wsem.at[k & (_NWSEM - 1)]).start()

    def wr_wait(k):
        v = pool.at[pl.ds(0, _OCT), pl.ds(0, _BT)]
        pltpu.make_async_copy(v, v, wsem.at[k & (_NWSEM - 1)]).wait()

    def blk(ls, j):
        return pool.at[ls, pl.ds(pl.multiple_of(j * _BT, _BT), _BT)]

    def fold(v):
        n = v.shape[0]
        while n > AW:
            n //= 2
            v = v[:n] + v[n:]
        return v

    def pass1(lg, j, acc):
        for s in range(_SPG):
            acc = acc + fold(blk(lg * _SPG + s, j)[...].astype(f32))
        return acc

    def pass2(lg, j, mean, acc):
        for s in range(_SPG):
            d = blk(lg * _SPG + s, j)[...].astype(f32) - mean
            acc = acc + fold(d * d)
        return acc

    def total(acc):
        a = acc[0]
        for i in range(1, AW):
            a = a + acc[i]
        return jnp.sum(jnp.sum(a, axis=1, keepdims=True), axis=0, keepdims=True) * (1.0 / n_group)

    def fin_mean(lg, acc):
        stat_smem[2 * lg] = total(acc)[0, 0]

    def fin_rstd(lg, acc):
        stat_smem[2 * lg + 1] = lax.rsqrt(total(acc) + _EPS)[0, 0]

    def normalize(bs, o, j):
        c0 = ((_shr(bs, 3) + o) & (oct_per_batch - 1)) * ch_per_oct
        row = _shr(c0, 7)
        col0 = (c0 & 127) + _shr(j, lbpc)
        for q in range(2):
            mean = stat_smem[4 * o + 2 * q]
            rstd = stat_smem[4 * o + 2 * q + 1]
            for s in range(q * _SPG, (q + 1) * _SPG):
                scale = rstd * gb_smem[row, col0 + s * cps]
                bias = gb_smem[8 + row, col0 + s * cps]
                ref = blk(o * _OCT + s, j)
                ref[...] = ((ref[...].astype(f32) - mean) * scale + bias).astype(pool.dtype)

    zeros = lambda: jnp.zeros((AW, 8, 128), f32)

    def start_round_reads(bs, first=0):
        for t in range(first, dr * rw):
            rd_start(bs, t // rw, t % rw)

    rd_start(0, 0, 0)
    gcp = pltpu.make_async_copy(g_hbm, gb_vmem.at[0], psem.at[0])
    bcp = pltpu.make_async_copy(b_hbm, gb_vmem.at[1], psem.at[1])
    gcp.start(); bcp.start()
    start_round_reads(0, 1)
    gcp.wait(); bcp.wait()
    gbf_vmem[0:8, :] = gb_vmem[0].astype(f32)
    gbf_vmem[8:16, :] = gb_vmem[1].astype(f32)
    scp = pltpu.make_async_copy(gbf_vmem, gb_smem, psem.at[2])
    scp.start()

    n_p2_units = -(-4 // rw)

    def round_body(r, carry):
        bs = r * (n_full * spu)
        n = jnp.where(r == n_rounds - 1, n_last, n_full) if n_last != n_full else n_full
        nw = n * spu // _OCT
        NW = nw * nb

        for q in range(rw):
            rd_wait(0, q)
            rd_start(bs, dr, q)

        def read_unit(u, pu, with_p2, last):
            if with_p2:
                ms = [stat_smem[2 * (pu * rw + q)] for q in range(rw)]
            def step(j, accs, wait, issue, start_writes_after=None):
                accs = list(accs)
                p = u * nb + j + 1
                for q in range(rw):
                    if wait:
                        rd_wait(p, q)
                    if issue:
                        rd_start(bs, p + dr, q)
                    if start_writes_after == q:
                        for k in range(dw):
                            wr_start(bs, k)
                    if do_compute:
                        accs[q] = pass1(u * rw + q, j, accs[q])
                        if with_p2:
                            accs[rw + q] = pass2(pu * rw + q, j, ms[q], accs[rw + q])
                return tuple(accs)
            def body(j, accs):
                accs = step(j, accs, True, True)
                if last and do_compute:
                    @pl.when(j < dw)
                    def _():
                        normalize(bs, 0, j)
                return accs
            accs = tuple(zeros() for _ in range(2 * rw if with_p2 else rw))
            accs = lax.fori_loop(0, nb - 1 - dr if last else nb, body, accs)
            if last:
                tsw = nb * rw - 1 - r2w_lead
                for j in range(nb - 1 - dr, nb):
                    row = j + 1
                    accs = step(j, accs, row < nb, False, (tsw - rw * row) if tsw // rw == row else None)
            if do_compute:
                for q in range(rw):
                    fin_mean(u * rw + q, accs[q])
                    if with_p2:
                        fin_rstd(pu * rw + q, accs[rw + q])

        def write_window(o, po, with_p2, j_start):
            if with_p2:
                ms = (stat_smem[4 * po], stat_smem[4 * po + 2])
            def body(j, accs):
                k = o * nb + j
                if do_compute:
                    normalize(bs, o, j)
                wr_wait(k - dw)
                wr_start(bs, k)
                if with_p2 and do_compute:
                    accs = (pass2(2 * po, j, ms[0], accs[0]), pass2(2 * po + 1, j, ms[1], accs[1]))
                return accs
            accs = lax.fori_loop(j_start, nb, body, tuple(zeros() for _ in range(2 if with_p2 else 0)))
            if with_p2 and do_compute:
                fin_rstd(2 * po, accs[0]); fin_rstd(2 * po + 1, accs[1])

        def rloop(u, c):
            has = jnp.logical_and(u >= 1, u <= n_p2_units)
            @pl.when(has)
            def _():
                read_unit(u, u - 1, True, False)
            @pl.when(jnp.logical_not(has))
            def _():
                read_unit(u, u - 1, False, False)
            return c
        lax.fori_loop(0, n - 1, rloop, 0)
        @pl.when(r == 0)
        def _():
            scp.wait()
        read_unit(n - 1, None, False, True)

        first_w_p2 = n_p2_units * rw // 2 - 1
        def wloop(o, c):
            has = jnp.logical_and(o >= max(first_w_p2, 1), o <= nw - 2)
            @pl.when(has)
            def _():
                write_window(o, o + 1, True, 0)
            @pl.when(jnp.logical_not(has))
            def _():
                write_window(o, o + 1, False, jnp.where(o == 0, dw, 0))
            return c
        lax.fori_loop(0, nw, wloop, 0)

        for i in range(dw):
            wr_wait(NW - dw + i)
            if i == dw - 1 - w2r_lead:
                @pl.when(r < n_rounds - 1)
                def _():
                    start_round_reads(bs + n_full * spu)
        return carry

    lax.fori_loop(0, n_rounds, round_body, 0)


def make(rw=2, n_full=11, sh=3, dr=5, dw=6, r2w_lead=4, w2r_lead=1, wsplit=2, do_compute=True, vmem_mb=110,
         nobc=False):
    @jax.jit
    def f(x, g, b):
        B, C, H, W = x.shape
        cpg = C // _G
        cps = cpg // _SPG
        NS = B * _G * _SPG
        rgs = cps * H // 8
        wt = W // 128
        tps = rgs * wt
        n_units = B * _G // rw
        n_rounds = -(-n_units // n_full)
        n_last = n_units - (n_rounds - 1) * n_full
        assert rw in (2, 4) and n_last >= -(-4 // rw) + 2
        assert rw * dr <= _NRSEM and dw <= _NWSEM and r2w_lead < rw * dr and w2r_lead < dw
        xl = x.reshape(NS * rgs, 8, wt, 128).transpose(0, 2, 1, 3).reshape(NS, tps, 8, 128)
        out = pl.pallas_call(
            functools.partial(_gn_kernel, n_rounds=n_rounds, n_full=n_full, n_last=n_last, tps=tps, cps=cps,
                              rw=rw, sh=sh, dr=dr, dw=dw, r2w_lead=r2w_lead, w2r_lead=w2r_lead, wsplit=wsplit,
                              do_compute=do_compute),
            in_specs=[pl.BlockSpec(memory_space=pl.ANY)] * 3,
            out_specs=pl.BlockSpec(memory_space=pl.ANY),
            out_shape=jax.ShapeDtypeStruct(xl.shape, x.dtype),
            scratch_shapes=[
                pltpu.VMEM((n_full * rw * _SPG, tps, 8, 128), x.dtype),
                pltpu.VMEM((2, 8, 128), g.dtype),
                pltpu.VMEM((16, 128), jnp.float32),
                pltpu.SMEM((16, 128), jnp.float32),
                pltpu.SMEM((2 * rw * n_full,), jnp.float32),
                pltpu.SemaphoreType.DMA((_NRSEM,)),
                pltpu.SemaphoreType.DMA((_NWSEM,)),
                pltpu.SemaphoreType.DMA((3,)),
            ],
            compiler_params=pltpu.CompilerParams(vmem_limit_bytes=vmem_mb * 1024 * 1024,
                                                 disable_bounds_checks=nobc),
        )(xl, g.reshape(8, 128), b.reshape(8, 128))
        return out.reshape(NS * rgs, wt, 8, 128).transpose(0, 2, 1, 3).reshape(B, C, H, W)
    return f


_impl = make()


@jax.jit
def pallas_standalone__groupnorm__prompt_kernel(x, g, b):
    return _impl(x, g, b)
```

```python
import functools

import jax
import jax.numpy as jnp
from jax import lax
import jax.experimental.pallas as pl
import jax.experimental.pallas.tpu as pltpu

_G = 32
_EPS = 1e-5
_SPG = 4
_BT = 16
_AW = 2
_NRSEM = 32
_NWSEM = 16


def _log2(n):
    l = n.bit_length() - 1
    assert 1 << l == n, n
    return l


def _shr(x, n):
    if isinstance(x, int):
        return x >> n
    return lax.shift_right_logical(x, jnp.int32(n))


def _branch(cond, if_true, if_false):
    if isinstance(cond, bool):
        (if_true if cond else if_false)()
    else:
        pl.when(jnp.logical_not(cond))(if_false)
        pl.when(cond)(if_true)


def _gn_kernel(x_hbm, g_hbm, b_hbm, o_hbm,
               pool, gb_vmem, gbf_vmem, gb_smem, stat_smem, rsem, wsem, psem,
               *, n_rounds, n_full, n_last, tps, cps, rw, parts, sh, dr, dh, dw, r2w_lead, w2r_lead,
               wsplit, w1, w2, wins_full, wins_last, do_compute):
    nb = tps // _BT
    lnb = _log2(nb)
    lbpc = _log2(nb // cps)
    slabs_per_batch = _G * _SPG
    n_group = _SPG * tps * 8 * 128
    spu = rw * _SPG
    npt = len(parts)
    poff = [sum(parts[:i]) for i in range(npt)]
    assert sum(parts) == spu
    f32 = jnp.float32

    def rd_copies(bs, p, q, head, prios):
        ls = _shr(p, lnb) * spu + poff[q]
        ns = parts[q]
        sem = rsem.at[(p * npt + q) & (_NRSEM - 1)]

        def cp(s0, n, t0, nt):
            return pltpu.make_async_copy(x_hbm.at[pl.ds(bs + ls + s0, n), pl.ds(t0, nt)],
                                         pool.at[pl.ds(ls + s0, n), pl.ds(t0, nt)], sem)
        if head:
            spec = ([(0, 1, 0, _BT - sh)], [(0, ns, tps - sh, sh), (1, ns - 1, 0, _BT - sh)])
        else:
            t0 = (p & (nb - 1)) * _BT - sh
            spec = ([(0, 1, t0, _BT)], [(1, ns - 1, t0, _BT)])
        return [cp(*a) for prio in prios for a in spec[prio]]

    def is_head(p):
        return sh > 0 and (p & (nb - 1)) == 0

    def rd_start(bs, p, q, prio, may_be_head=True):
        def go(head):
            for c in rd_copies(bs, p, q, head, (prio,)):
                c.start(priority=prio)
        _branch(may_be_head and is_head(p), lambda: go(True), lambda: go(False))

    def rd_wait(bs, p, q, may_be_head=True):
        def go(head):
            for c in rd_copies(bs, p, q, head, (0, 1)):
                c.wait()
        _branch(may_be_head and is_head(p), lambda: go(True), lambda: go(False))

    def start_round_reads(bs):
        for t in range(dr * npt):
            if t < dh * npt:
                rd_start(bs, t // npt, t % npt, 0)
            rd_start(bs, t // npt, t % npt, 1)

    def wr_copies(bs, ls, ns, j, k):
        ht = _BT // wsplit
        return [pltpu.make_async_copy(pool.at[pl.ds(ls, ns), pl.ds(j * _BT + h * ht, ht)],
                                      o_hbm.at[pl.ds(bs + ls, ns), pl.ds(j * _BT + h * ht, ht)],
                                      wsem.at[k & (_NWSEM - 1)]) for h in range(wsplit)]

    def wr_start(*a):
        for c in wr_copies(*a):
            c.start()

    def wr_wait(*a):
        for c in wr_copies(*a):
            c.wait()

    def blk(ls, j):
        return pool.at[ls, pl.ds(pl.multiple_of(j * _BT, _BT), _BT)]

    def fold(v):
        n = v.shape[0]
        while n > _AW:
            n //= 2
            v = v[:n] + v[n:]
        return v

    def add_sum(ls, j, acc):
        return acc + fold(blk(ls, j)[...].astype(f32))

    def add_sqdev(ls, j, mean, acc):
        d = blk(ls, j)[...].astype(f32) - mean
        return acc + fold(d * d)

    def group_avg(acc):
        a = acc[0]
        for i in range(1, _AW):
            a = a + acc[i]
        return jnp.sum(jnp.sum(a, axis=1, keepdims=True), axis=0, keepdims=True) * (1.0 / n_group)

    def put_mean(lg, acc):
        stat_smem[2 * lg] = group_avg(acc)[0, 0]

    def put_rstd(lg, acc):
        stat_smem[2 * lg + 1] = lax.rsqrt(group_avg(acc) + _EPS)[0, 0]

    def normalize(bs, ls0, ns, j):
        cj = _shr(j, lbpc)
        for s in range(ns):
            ls = ls0 + s
            st = _shr(ls, _log2(_SPG)) * 2
            mean = stat_smem[st]
            rstd = stat_smem[st + 1]
            c = ((bs + ls) & (slabs_per_batch - 1)) * cps + cj
            row = _shr(c, 7)
            col = c & 127
            scale = rstd * gb_smem[row, col]
            bias = gb_smem[8 + row, col]
            ref = blk(ls, j)
            ref[...] = ((ref[...].astype(f32) - mean) * scale + bias).astype(pool.dtype)

    def zeros(n):
        return tuple(jnp.zeros((_AW, 8, 128), f32) for _ in range(n))

    start_round_reads(0)
    gcp = pltpu.make_async_copy(g_hbm, gb_vmem.at[0], psem.at[0])
    bcp = pltpu.make_async_copy(b_hbm, gb_vmem.at[1], psem.at[1])
    gcp.start()
    bcp.start()
    scp = pltpu.make_async_copy(gbf_vmem, gb_smem, psem.at[2])

    n_p2_units = -(-4 // rw)

    def round_body(r, carry):
        bs = r * (n_full * spu)
        is_last = r == n_rounds - 1
        n = jnp.where(is_last, n_last, n_full)
        na = jnp.where(is_last, wins_last[0], wins_full[0])
        nb2 = jnp.where(is_last, wins_last[1], wins_full[1])
        n_pairs = n * (rw // 2)

        for q in range(npt):
            rd_wait(bs, 0, q)
            rd_start(bs, dh, q, 0)
            rd_start(bs, dr, q, 1)

        @pl.when(r == 0)
        def _():
            gcp.wait()
            bcp.wait()
            gbf_vmem[0:8, :] = gb_vmem[0].astype(f32)
            gbf_vmem[8:16, :] = gb_vmem[1].astype(f32)
            scp.start()

        def read_unit(u, pu, with_p2, last):
            if with_p2:
                ms = [stat_smem[2 * (pu * rw + g)] for g in range(rw)]

            def step(j, accs, wait, issue_hi, issue_lo, start_writes_after=None):
                accs = list(accs)
                p = u * nb + j + 1
                for q in range(npt):
                    if wait:
                        rd_wait(bs, p, q, not last)
                    if issue_hi:
                        rd_start(bs, p + dh, q, 0, not last)
                    if issue_lo:
                        rd_start(bs, p + dr, q, 1, not last)
                    if start_writes_after == q:
                        for k in range(dw):
                            wr_start(bs, 0, w1, k, k)
                    if do_compute:
                        for s in range(poff[q], poff[q] + parts[q]):
                            g = s // _SPG
                            accs[g] = add_sum(u * spu + s, j, accs[g])
                            if with_p2:
                                accs[rw + g] = add_sqdev(pu * spu + s, j, ms[g], accs[rw + g])
                return tuple(accs)

            def body(j, accs):
                accs = step(j, accs, True, True, True)
                if last and do_compute:
                    @pl.when(j < dw)
                    def _():
                        normalize(bs, 0, w1, j)
                return accs

            accs = lax.fori_loop(0, nb - 1 - dr if last else nb, body, zeros(2 * rw if with_p2 else rw))
            if last:
                tsw = nb * npt - 1 - r2w_lead
                for j in range(nb - 1 - dr, nb):
                    row = j + 1
                    accs = step(j, accs, row < nb, row + dh < nb, False,
                                (tsw - npt * row) if tsw // npt == row else None)
            if do_compute:
                for g in range(rw):
                    put_mean(u * rw + g, accs[g])
                    if with_p2:
                        put_rstd(pu * rw + g, accs[rw + g])

        def rloop(u, c):
            _branch(jnp.logical_and(u >= 1, u <= n_p2_units),
                    lambda: read_unit(u, u - 1, True, False),
                    lambda: read_unit(u, None, False, False))
            return c

        lax.fori_loop(0, n - 1, rloop, 0)

        @pl.when(r == 0)
        def _():
            scp.wait()

        read_unit(n - 1, None, False, True)

        def write_window(o, ls0, ns, po, j_start, prev_is_w1=None):
            with_p2 = po is not None
            if with_p2:
                ms = (stat_smem[4 * po], stat_smem[4 * po + 2])

            def body(j, accs):
                k = o * nb + j
                if do_compute:
                    normalize(bs, ls0, ns, j)
                back = j < dw
                jo = (j - dw) & (nb - 1)
                same = lambda: wr_wait(bs, jnp.where(back, ls0 - ns, ls0), ns, jo, k - dw)
                if prev_is_w1 is None:
                    same()
                else:
                    _branch(jnp.logical_and(prev_is_w1, back),
                            lambda: wr_wait(bs, ls0 - w1, w1, jo, k - dw), same)
                wr_start(bs, ls0, ns, j, k)
                if with_p2 and do_compute:
                    accs = list(accs)
                    for s in range(2 * _SPG):
                        g = s // _SPG
                        accs[g] = add_sqdev(po * 2 * _SPG + s, j, ms[g], accs[g])
                    accs = tuple(accs)
                return accs

            accs = lax.fori_loop(j_start, nb, body, zeros(2 if with_p2 else 0))
            if with_p2 and do_compute:
                put_rstd(2 * po, accs[0])
                put_rstd(2 * po + 1, accs[1])

        def wloop(o, c):
            _branch(jnp.logical_and(o >= 1, o <= n_pairs - 2),
                    lambda: write_window(o, o * w1, w1, o + 1, 0),
                    lambda: write_window(o, o * w1, w1, None, jnp.where(o == 0, dw, 0)))
            return c

        lax.fori_loop(0, na, wloop, 0)

        def wloop2(i, c):
            write_window(na + i, na * w1 + i * w2, w2, None, 0, i == 0)
            return c

        if max(wins_full[1], wins_last[1]) > 0:
            lax.fori_loop(0, nb2, wloop2, 0)

        n_slabs = n * spu
        n_chunks = (na + nb2) * nb
        if min(wins_full[1], wins_last[1]) > 0:
            ends_w2 = True
        elif max(wins_full[1], wins_last[1]) == 0:
            ends_w2 = False
        else:
            ends_w2 = nb2 > 0
        for i in range(dw):
            _branch(ends_w2,
                    lambda: wr_wait(bs, n_slabs - w2, w2, nb - dw + i, n_chunks - dw + i),
                    lambda: wr_wait(bs, n_slabs - w1, w1, nb - dw + i, n_chunks - dw + i))
            if i == dw - 1 - w2r_lead:
                @pl.when(r < n_rounds - 1)
                def _():
                    start_round_reads(bs + n_full * spu)
        return carry

    lax.fori_loop(0, n_rounds, round_body, 0)


def make(rw=4, parts=(2, 3, 3, 2, 3, 3), n_full=6, sh=3, dr=3, dh=2, dw=8, r2w_lead=7, w2r_lead=1, wsplit=2,
         w1=6, w2=8, do_compute=True, vmem_mb=110, debug_checks=False):
    def split_windows(s):
        for b2 in range(s // w2 + 1):
            if (s - b2 * w2) % w1 == 0:
                return ((s - b2 * w2) // w1, b2)
        raise ValueError(s)

    @jax.jit
    def f(x, g, b):
        B, C, H, W = x.shape
        cpg = C // _G
        cps = cpg // _SPG
        n_slabs = B * _G * _SPG
        rgs = cps * H // 8
        wt = W // 128
        tps = rgs * wt
        n_units = B * _G // rw
        n_rounds = -(-n_units // n_full)
        n_last = n_units - (n_rounds - 1) * n_full
        assert C == 1024 and H % 8 == 0 and W % 128 == 0 and (tps // _BT) % cps == 0
        assert rw in (2, 4) and n_last >= -(-4 // rw) + 2 and 0 <= sh < _BT and 1 <= dh <= dr
        assert len(parts) * dr <= _NRSEM and dw <= _NWSEM and r2w_lead < len(parts) * dr and w2r_lead < dw
        wins_full = split_windows(n_full * rw * _SPG)
        wins_last = split_windows(n_last * rw * _SPG)
        for nn, ww in ((n_full, wins_full), (n_last, wins_last)):
            assert nn * rw // 2 - 2 < ww[0] and w1 <= 8
        xl = x.reshape(n_slabs * rgs, 8, wt, 128).transpose(0, 2, 1, 3).reshape(n_slabs, tps, 8, 128)
        out = pl.pallas_call(
            functools.partial(_gn_kernel, n_rounds=n_rounds, n_full=n_full, n_last=n_last, tps=tps, cps=cps,
                              rw=rw, parts=parts, sh=sh, dr=dr, dh=dh, dw=dw, r2w_lead=r2w_lead,
                              w2r_lead=w2r_lead, wsplit=wsplit, w1=w1, w2=w2, wins_full=wins_full,
                              wins_last=wins_last, do_compute=do_compute),
            in_specs=[pl.BlockSpec(memory_space=pl.ANY)] * 3,
            out_specs=pl.BlockSpec(memory_space=pl.ANY),
            out_shape=jax.ShapeDtypeStruct(xl.shape, x.dtype),
            scratch_shapes=[
                pltpu.VMEM((n_full * rw * _SPG, tps, 8, 128), x.dtype),
                pltpu.VMEM((2, 8, 128), g.dtype),
                pltpu.VMEM((16, 128), jnp.float32),
                pltpu.SMEM((16, 128), jnp.float32),
                pltpu.SMEM((2 * rw * n_full,), jnp.float32),
                pltpu.SemaphoreType.DMA((_NRSEM,)),
                pltpu.SemaphoreType.DMA((_NWSEM,)),
                pltpu.SemaphoreType.DMA((3,)),
            ],
            compiler_params=pltpu.CompilerParams(vmem_limit_bytes=vmem_mb * 1024 * 1024,
                                                 disable_bounds_checks=not debug_checks,
                                                 disable_semaphore_checks=not debug_checks),
        )(xl, g.reshape(8, 128), b.reshape(8, 128))
        return out.reshape(n_slabs * rgs, wt, 8, 128).transpose(0, 2, 1, 3).reshape(B, C, H, W)
    return f


_impl = make()


@jax.jit
def pallas_standalone__groupnorm__prompt_kernel(x, g, b):
    return _impl(x, g, b)
```

```python
import functools

import jax
import jax.numpy as jnp
from jax import lax
import jax.experimental.pallas as pl
import jax.experimental.pallas.tpu as pltpu

_G = 32
_EPS = 1e-5
_SPG = 4
_BT = 16
_AW = 2
_GPU = 4
_SPU = _GPU * _SPG
_PARTS = (2, 3, 3, 2, 3, 3)
_UNITS_PER_ROUND = 6
_SH = 3
_DR = 3
_DH = 2
_DW = 8
_R2W = 7
_W2R = 1
_WSPLIT = 2
_W1, _W2 = 6, 8
_NRSEM = 32
_NWSEM = 16


def _log2(n):
    l = n.bit_length() - 1
    assert 1 << l == n, n
    return l


def _shr(x, n):
    if isinstance(x, int):
        return x >> n
    return lax.shift_right_logical(x, jnp.int32(n))


def _branch(cond, if_true, if_false):
    if isinstance(cond, bool):
        (if_true if cond else if_false)()
    else:
        pl.when(jnp.logical_not(cond))(if_false)
        pl.when(cond)(if_true)


def _split_windows(n_slabs):
    for n2 in range(n_slabs // _W2 + 1):
        if (n_slabs - n2 * _W2) % _W1 == 0:
            return (n_slabs - n2 * _W2) // _W1, n2
    raise ValueError(n_slabs)


def _gn_kernel(x_hbm, g_hbm, b_hbm, o_hbm,
               pool, gb_vmem, gbf_vmem, gb_smem, stat_smem, rsem, wsem, psem,
               *, n_rounds, n_full, n_last, tps, cps):
    nb = tps // _BT
    lnb = _log2(nb)
    lbpc = _log2(nb // cps)
    slabs_per_image = _G * _SPG
    n_group = _SPG * tps * 8 * 128
    npt = len(_PARTS)
    poff = [sum(_PARTS[:i]) for i in range(npt)]
    wins_full = _split_windows(n_full * _SPU)
    wins_last = _split_windows(n_last * _SPU)
    f32 = jnp.float32

    def rd_copies(bs, p, q, head, prios):
        ls = _shr(p, lnb) * _SPU + poff[q]
        ns = _PARTS[q]
        sem = rsem.at[(p * npt + q) & (_NRSEM - 1)]
        if head:
            spec = ([(0, 1, 0, _BT - _SH)], [(0, ns, tps - _SH, _SH), (1, ns - 1, 0, _BT - _SH)])
        else:
            t0 = (p & (nb - 1)) * _BT - _SH
            spec = ([(0, 1, t0, _BT)], [(1, ns - 1, t0, _BT)])
        return [pltpu.make_async_copy(x_hbm.at[pl.ds(bs + ls + s0, n), pl.ds(t, nt)],
                                      pool.at[pl.ds(ls + s0, n), pl.ds(t, nt)], sem)
                for prio in prios for (s0, n, t, nt) in spec[prio]]

    def rd_start(bs, p, q, prio, may_be_head=True):
        def go(head):
            for c in rd_copies(bs, p, q, head, (prio,)):
                c.start(priority=prio)
        _branch(may_be_head and (p & (nb - 1)) == 0, lambda: go(True), lambda: go(False))

    def rd_wait(bs, p, q, may_be_head=True):
        def go(head):
            for c in rd_copies(bs, p, q, head, (0, 1)):
                c.wait()
        _branch(may_be_head and (p & (nb - 1)) == 0, lambda: go(True), lambda: go(False))

    def start_round_reads(bs):
        for t in range(_DR * npt):
            if t < _DH * npt:
                rd_start(bs, t // npt, t % npt, 0)
            rd_start(bs, t // npt, t % npt, 1)

    def wr_copies(bs, ls, ns, j, k):
        ht = _BT // _WSPLIT
        return [pltpu.make_async_copy(pool.at[pl.ds(ls, ns), pl.ds(j * _BT + h * ht, ht)],
                                      o_hbm.at[pl.ds(bs + ls, ns), pl.ds(j * _BT + h * ht, ht)],
                                      wsem.at[k & (_NWSEM - 1)]) for h in range(_WSPLIT)]

    def wr_start(*a):
        for c in wr_copies(*a):
            c.start()

    def wr_wait(*a):
        for c in wr_copies(*a):
            c.wait()

    def blk(ls, j):
        return pool.at[ls, pl.ds(pl.multiple_of(j * _BT, _BT), _BT)]

    def fold(v):
        n = v.shape[0]
        while n > _AW:
            n //= 2
            v = v[:n] + v[n:]
        return v

    def add_sum(ls, j, acc):
        return acc + fold(blk(ls, j)[...].astype(f32))

    def add_sqdev(ls, j, mean, acc):
        d = blk(ls, j)[...].astype(f32) - mean
        return acc + fold(d * d)

    def group_avg(acc):
        a = acc[0]
        for i in range(1, _AW):
            a = a + acc[i]
        return jnp.sum(jnp.sum(a, axis=1, keepdims=True), axis=0, keepdims=True) * (1.0 / n_group)

    def put_mean(lg, acc):
        stat_smem[2 * lg] = group_avg(acc)[0, 0]

    def put_rstd(lg, acc):
        stat_smem[2 * lg + 1] = lax.rsqrt(group_avg(acc) + _EPS)[0, 0]

    def normalize(bs, ls0, ns, j):
        cj = _shr(j, lbpc)
        for s in range(ns):
            ls = ls0 + s
            st = _shr(ls, _log2(_SPG)) * 2
            mean = stat_smem[st]
            rstd = stat_smem[st + 1]
            c = ((bs + ls) & (slabs_per_image - 1)) * cps + cj
            row = _shr(c, 7)
            col = c & 127
            scale = rstd * gb_smem[row, col]
            bias = gb_smem[8 + row, col]
            ref = blk(ls, j)
            ref[...] = ((ref[...].astype(f32) - mean) * scale + bias).astype(pool.dtype)

    def zeros(n):
        return tuple(jnp.zeros((_AW, 8, 128), f32) for _ in range(n))

    start_round_reads(0)
    gcp = pltpu.make_async_copy(g_hbm, gb_vmem.at[0], psem.at[0])
    bcp = pltpu.make_async_copy(b_hbm, gb_vmem.at[1], psem.at[1])
    gcp.start()
    bcp.start()
    scp = pltpu.make_async_copy(gbf_vmem, gb_smem, psem.at[2])

    def round_body(r, carry):
        bs = r * (n_full * _SPU)
        is_last = r == n_rounds - 1
        n = jnp.where(is_last, n_last, n_full)
        n1 = jnp.where(is_last, wins_last[0], wins_full[0])
        n2 = jnp.where(is_last, wins_last[1], wins_full[1])
        n_pairs = n * (_GPU // 2)

        for q in range(npt):
            rd_wait(bs, 0, q)
            rd_start(bs, _DH, q, 0)
            rd_start(bs, _DR, q, 1)

        @pl.when(r == 0)
        def _():
            gcp.wait()
            bcp.wait()
            gbf_vmem[0:8, :] = gb_vmem[0].astype(f32)
            gbf_vmem[8:16, :] = gb_vmem[1].astype(f32)
            scp.start()

        def read_unit(u, var_unit, last):
            with_var = var_unit is not None
            if with_var:
                means = [stat_smem[2 * (var_unit * _GPU + g)] for g in range(_GPU)]

            def step(j, accs, wait, issue_hi, issue_lo, start_writes_after=None):
                accs = list(accs)
                p = u * nb + j + 1
                for q in range(npt):
                    if wait:
                        rd_wait(bs, p, q, not last)
                    if issue_hi:
                        rd_start(bs, p + _DH, q, 0, not last)
                    if issue_lo:
                        rd_start(bs, p + _DR, q, 1, not last)
                    if start_writes_after == q:
                        for k in range(_DW):
                            wr_start(bs, 0, _W1, k, k)
                    for s in range(poff[q], poff[q] + _PARTS[q]):
                        g = s // _SPG
                        accs[g] = add_sum(u * _SPU + s, j, accs[g])
                        if with_var:
                            accs[_GPU + g] = add_sqdev(var_unit * _SPU + s, j, means[g], accs[_GPU + g])
                return tuple(accs)

            def body(j, accs):
                accs = step(j, accs, True, True, True)
                if last:
                    @pl.when(j < _DW)
                    def _():
                        normalize(bs, 0, _W1, j)
                return accs

            accs = lax.fori_loop(0, nb - 1 - _DR if last else nb, body, zeros(2 * _GPU if with_var else _GPU))
            if last:
                tsw = nb * npt - 1 - _R2W
                for j in range(nb - 1 - _DR, nb):
                    row = j + 1
                    accs = step(j, accs, row < nb, row + _DH < nb, False,
                                (tsw - npt * row) if tsw // npt == row else None)
            for g in range(_GPU):
                put_mean(u * _GPU + g, accs[g])
                if with_var:
                    put_rstd(var_unit * _GPU + g, accs[_GPU + g])

        def read_loop(u, c):
            _branch(u == 1, lambda: read_unit(u, u - 1, False), lambda: read_unit(u, None, False))
            return c

        lax.fori_loop(0, n - 1, read_loop, 0)

        @pl.when(r == 0)
        def _():
            scp.wait()

        read_unit(n - 1, None, True)

        def write_window(o, ls0, ns, var_pair, j_start, prev_is_w1=None):
            with_var = var_pair is not None
            if with_var:
                means = (stat_smem[4 * var_pair], stat_smem[4 * var_pair + 2])

            def body(j, accs):
                k = o * nb + j
                normalize(bs, ls0, ns, j)
                back = j < _DW
                jo = (j - _DW) & (nb - 1)

                def wait_same():
                    wr_wait(bs, jnp.where(back, ls0 - ns, ls0), ns, jo, k - _DW)

                if prev_is_w1 is None:
                    wait_same()
                else:
                    _branch(jnp.logical_and(prev_is_w1, back),
                            lambda: wr_wait(bs, ls0 - _W1, _W1, jo, k - _DW), wait_same)
                wr_start(bs, ls0, ns, j, k)
                if with_var:
                    accs = list(accs)
                    for s in range(2 * _SPG):
                        g = s // _SPG
                        accs[g] = add_sqdev(var_pair * 2 * _SPG + s, j, means[g], accs[g])
                    accs = tuple(accs)
                return accs

            accs = lax.fori_loop(j_start, nb, body, zeros(2 if with_var else 0))
            if with_var:
                put_rstd(2 * var_pair, accs[0])
                put_rstd(2 * var_pair + 1, accs[1])

        def write_loop1(o, c):
            _branch(jnp.logical_and(o >= 1, o <= n_pairs - 2),
                    lambda: write_window(o, o * _W1, _W1, o + 1, 0),
                    lambda: write_window(o, o * _W1, _W1, None, jnp.where(o == 0, _DW, 0)))
            return c

        lax.fori_loop(0, n1, write_loop1, 0)

        def write_loop2(i, c):
            write_window(n1 + i, n1 * _W1 + i * _W2, _W2, None, 0, i == 0)
            return c

        lax.fori_loop(0, n2, write_loop2, 0)

        n_slabs = n * _SPU
        n_chunks = (n1 + n2) * nb
        for i in range(_DW):
            _branch(n2 > 0,
                    lambda: wr_wait(bs, n_slabs - _W2, _W2, nb - _DW + i, n_chunks - _DW + i),
                    lambda: wr_wait(bs, n_slabs - _W1, _W1, nb - _DW + i, n_chunks - _DW + i))
            if i == _DW - 1 - _W2R:
                @pl.when(r < n_rounds - 1)
                def _():
                    start_round_reads(bs + n_full * _SPU)
        return carry

    lax.fori_loop(0, n_rounds, round_body, 0)


@jax.jit
def pallas_standalone__groupnorm__prompt_kernel(x: jax.Array, g: jax.Array, b: jax.Array):
    B, C, H, W = x.shape
    cps = C // _G // _SPG
    n_slabs = B * _G * _SPG
    rgs = cps * H // 8
    wt = W // 128
    tps = rgs * wt
    n_units = B * _G // _GPU
    n_full = _UNITS_PER_ROUND
    n_rounds = -(-n_units // n_full)
    n_last = n_units - (n_rounds - 1) * n_full
    nb = tps // _BT
    assert C == 8 * 128 and H % 8 == 0 and W % 128 == 0 and nb % cps == 0 and _DW <= nb - 1 - _DR
    assert n_last >= 3 and sum(_PARTS) == _SPU and len(_PARTS) * _DR <= _NRSEM and _DW <= _NWSEM
    for nn in (n_full, n_last):
        assert nn * _GPU // 2 - 2 < _split_windows(nn * _SPU)[0]

    xl = x.reshape(n_slabs * rgs, 8, wt, 128).transpose(0, 2, 1, 3).reshape(n_slabs, tps, 8, 128)
    out = pl.pallas_call(
        functools.partial(_gn_kernel, n_rounds=n_rounds, n_full=n_full, n_last=n_last, tps=tps, cps=cps),
        in_specs=[pl.BlockSpec(memory_space=pl.ANY)] * 3,
        out_specs=pl.BlockSpec(memory_space=pl.ANY),
        out_shape=jax.ShapeDtypeStruct(xl.shape, x.dtype),
        scratch_shapes=[
            pltpu.VMEM((n_full * _SPU, tps, 8, 128), x.dtype),
            pltpu.VMEM((2, 8, 128), g.dtype),
            pltpu.VMEM((16, 128), jnp.float32),
            pltpu.SMEM((16, 128), jnp.float32),
            pltpu.SMEM((2 * _GPU * n_full,), jnp.float32),
            pltpu.SemaphoreType.DMA((_NRSEM,)),
            pltpu.SemaphoreType.DMA((_NWSEM,)),
            pltpu.SemaphoreType.DMA((3,)),
        ],
        compiler_params=pltpu.CompilerParams(
            vmem_limit_bytes=110 * 1024 * 1024,
            disable_bounds_checks=True,
            disable_semaphore_checks=True,
        ),
    )(xl, g.reshape(8, 128), b.reshape(8, 128))
    return out.reshape(n_slabs * rgs, wt, 8, 128).transpose(0, 2, 1, 3).reshape(B, C, H, W)
```

```python
import functools

import jax
import jax.numpy as jnp
from jax import lax
import jax.experimental.pallas as pl
import jax.experimental.pallas.tpu as pltpu

_G = 32
_EPS = 1e-5
_SPG = 4
_BT = 16
_AW = 4
_GPU = 4
_SPU = _GPU * _SPG
_PARTS = (2, 3, 3, 2, 3, 3)
_UNITS_PER_ROUND = 6
_SH = 3
_DR = 3
_DH = 2
_DW = 8
_R2W = 7
_W2R = 1
_WSPLIT = 2
_W1, _W2 = 6, 8
_NRSEM = 32
_NWSEM = 16


def _log2(n):
    l = n.bit_length() - 1
    assert 1 << l == n, n
    return l


def _shr(x, n):
    if isinstance(x, int):
        return x >> n
    return lax.shift_right_logical(x, jnp.int32(n))


def _branch(cond, if_true, if_false):
    if isinstance(cond, bool):
        (if_true if cond else if_false)()
    else:
        pl.when(jnp.logical_not(cond))(if_false)
        pl.when(cond)(if_true)


def _split_windows(n_slabs):
    for n2 in range(n_slabs // _W2 + 1):
        if (n_slabs - n2 * _W2) % _W1 == 0:
            return (n_slabs - n2 * _W2) // _W1, n2
    raise ValueError(n_slabs)


def _gn_kernel(x_hbm, g_hbm, b_hbm, o_hbm,
               pool, gb_vmem, gbf_vmem, gb_smem, stat_smem, rsem, wsem, psem,
               *, n_rounds, n_full, n_last, tps, cps):
    nb = tps // _BT
    lnb = _log2(nb)
    lbpc = _log2(nb // cps)
    slabs_per_image = _G * _SPG
    n_group = _SPG * tps * 8 * 128
    npt = len(_PARTS)
    poff = [sum(_PARTS[:i]) for i in range(npt)]
    wins_full = _split_windows(n_full * _SPU)
    wins_last = _split_windows(n_last * _SPU)
    f32 = jnp.float32

    def rd_copies(bs, p, q, head, prios):
        ls = _shr(p, lnb) * _SPU + poff[q]
        ns = _PARTS[q]
        sem = rsem.at[(p * npt + q) & (_NRSEM - 1)]
        if head:
            spec = ([(0, 1, 0, _BT - _SH)], [(0, ns, tps - _SH, _SH), (1, ns - 1, 0, _BT - _SH)])
        else:
            t0 = (p & (nb - 1)) * _BT - _SH
            spec = ([(0, 1, t0, _BT)], [(1, ns - 1, t0, _BT)])
        return [pltpu.make_async_copy(x_hbm.at[pl.ds(bs + ls + s0, n), pl.ds(t, nt)],
                                      pool.at[pl.ds(ls + s0, n), pl.ds(t, nt)], sem)
                for prio in prios for (s0, n, t, nt) in spec[prio]]

    def rd_start(bs, p, q, prio, may_be_head=True):
        def go(head):
            for c in rd_copies(bs, p, q, head, (prio,)):
                c.start(priority=prio)
        _branch(may_be_head and (p & (nb - 1)) == 0, lambda: go(True), lambda: go(False))

    def rd_wait(bs, p, q, may_be_head=True):
        def go(head):
            for c in rd_copies(bs, p, q, head, (0, 1)):
                c.wait()
        _branch(may_be_head and (p & (nb - 1)) == 0, lambda: go(True), lambda: go(False))

    def start_round_reads(bs):
        for t in range(_DR * npt):
            if t < _DH * npt:
                rd_start(bs, t // npt, t % npt, 0)
            rd_start(bs, t // npt, t % npt, 1)

    def wr_copies(bs, ls, ns, j, k):
        ht = _BT // _WSPLIT
        return [pltpu.make_async_copy(pool.at[pl.ds(ls, ns), pl.ds(j * _BT + h * ht, ht)],
                                      o_hbm.at[pl.ds(bs + ls, ns), pl.ds(j * _BT + h * ht, ht)],
                                      wsem.at[k & (_NWSEM - 1)]) for h in range(_WSPLIT)]

    def wr_start(*a):
        for c in wr_copies(*a):
            c.start()

    def wr_wait(*a):
        for c in wr_copies(*a):
            c.wait()

    def blk(ls, j):
        return pool.at[ls, pl.ds(pl.multiple_of(j * _BT, _BT), _BT)]

    def blks(ls, ns, j):
        v = pool[pl.ds(ls, ns), pl.ds(pl.multiple_of(j * _BT, _BT), _BT)].astype(f32)
        return v.reshape(ns * _BT // _AW, _AW, 8, 128)

    def add_sum(ls, ns, j, acc):
        return acc + jnp.sum(blks(ls, ns, j), axis=0)

    def add_sqdev(ls, ns, j, mean, acc):
        d = blks(ls, ns, j) - mean
        return acc + jnp.sum(d * d, axis=0)

    def group_avg(acc):
        a = acc[0]
        for i in range(1, _AW):
            a = a + acc[i]
        return jnp.sum(jnp.sum(a, axis=1, keepdims=True), axis=0, keepdims=True) * (1.0 / n_group)

    def put_mean(lg, acc):
        stat_smem[2 * lg] = group_avg(acc)[0, 0]

    def put_rstd(lg, acc):
        stat_smem[2 * lg + 1] = lax.rsqrt(group_avg(acc) + _EPS)[0, 0]

    def normalize(bs, ls0, ns, j):
        cj = _shr(j, lbpc)
        for s in range(ns):
            ls = ls0 + s
            st = _shr(ls, _log2(_SPG)) * 2
            mean = stat_smem[st]
            rstd = stat_smem[st + 1]
            c = ((bs + ls) & (slabs_per_image - 1)) * cps + cj
            row = _shr(c, 7)
            col = c & 127
            scale = rstd * gb_smem[row, col]
            bias = gb_smem[8 + row, col]
            ref = blk(ls, j)
            ref[...] = ((ref[...].astype(f32) - mean) * scale + bias).astype(pool.dtype)

    def zeros(n):
        return tuple(jnp.zeros((_AW, 8, 128), f32) for _ in range(n))

    start_round_reads(0)
    gcp = pltpu.make_async_copy(g_hbm, gb_vmem.at[0], psem.at[0])
    bcp = pltpu.make_async_copy(b_hbm, gb_vmem.at[1], psem.at[1])
    gcp.start()
    bcp.start()
    scp = pltpu.make_async_copy(gbf_vmem, gb_smem, psem.at[2])

    def round_body(r, carry):
        bs = r * (n_full * _SPU)
        is_last = r == n_rounds - 1
        n = jnp.where(is_last, n_last, n_full)
        n1 = jnp.where(is_last, wins_last[0], wins_full[0])
        n2 = jnp.where(is_last, wins_last[1], wins_full[1])
        n_pairs = n * (_GPU // 2)

        for q in range(npt):
            rd_wait(bs, 0, q)
            rd_start(bs, _DH, q, 0)
            rd_start(bs, _DR, q, 1)

        @pl.when(r == 0)
        def _():
            gcp.wait()
            bcp.wait()
            gbf_vmem[0:8, :] = gb_vmem[0].astype(f32)
            gbf_vmem[8:16, :] = gb_vmem[1].astype(f32)
            scp.start()

        def read_unit(u, var_unit, last):
            with_var = var_unit is not None
            if with_var:
                means = [stat_smem[2 * (var_unit * _GPU + g)] for g in range(_GPU)]

            def step(j, accs, near_end, wait=True, issue_hi=True, issue_lo=True, start_writes_after=None):
                accs = list(accs)
                p = u * nb + j + 1
                for q in range(npt):
                    if wait:
                        rd_wait(bs, p, q, near_end)
                    if issue_hi:
                        rd_start(bs, p + _DH, q, 0, near_end)
                    if issue_lo:
                        rd_start(bs, p + _DR, q, 1, near_end)
                    if start_writes_after == q:
                        for k in range(_DW):
                            wr_start(bs, 0, _W1, k, k)
                    for g in range(_GPU):
                        s0 = max(poff[q], g * _SPG)
                        ns = min(poff[q] + _PARTS[q], (g + 1) * _SPG) - s0
                        if ns > 0:
                            accs[g] = add_sum(u * _SPU + s0, ns, j, accs[g])
                            if with_var:
                                accs[_GPU + g] = add_sqdev(var_unit * _SPU + s0, ns, j, means[g], accs[_GPU + g])
                return tuple(accs)

            def body(j, accs):
                accs = step(j, accs, False)
                if last:
                    @pl.when(j < _DW)
                    def _():
                        normalize(bs, 0, _W1, j)
                return accs

            accs = lax.fori_loop(0, nb - 1 - _DR, body, zeros(2 * _GPU if with_var else _GPU))
            if last:
                tsw = nb * npt - 1 - _R2W
                for j in range(nb - 1 - _DR, nb):
                    row = j + 1
                    accs = step(j, accs, False, row < nb, row + _DH < nb, False,
                                (tsw - npt * row) if tsw // npt == row else None)
            else:
                accs = lax.fori_loop(nb - 1 - _DR, nb, lambda j, a: step(j, a, True), accs)
            for g in range(_GPU):
                put_mean(u * _GPU + g, accs[g])
                if with_var:
                    put_rstd(var_unit * _GPU + g, accs[_GPU + g])

        def read_loop(u, c):
            _branch(u == 1, lambda: read_unit(u, u - 1, False), lambda: read_unit(u, None, False))
            return c

        lax.fori_loop(0, n - 1, read_loop, 0)

        @pl.when(r == 0)
        def _():
            scp.wait()

        read_unit(n - 1, None, True)

        def write_window(o, ls0, ns, var_pair, j_start, prev_is_w1=None):
            with_var = var_pair is not None
            if with_var:
                means = (stat_smem[4 * var_pair], stat_smem[4 * var_pair + 2])

            def body(j, accs):
                k = o * nb + j
                normalize(bs, ls0, ns, j)
                back = j < _DW
                jo = (j - _DW) & (nb - 1)

                def wait_same():
                    wr_wait(bs, jnp.where(back, ls0 - ns, ls0), ns, jo, k - _DW)

                if prev_is_w1 is None:
                    wait_same()
                else:
                    _branch(jnp.logical_and(prev_is_w1, back),
                            lambda: wr_wait(bs, ls0 - _W1, _W1, jo, k - _DW), wait_same)
                wr_start(bs, ls0, ns, j, k)
                if with_var:
                    accs = tuple(add_sqdev((var_pair * 2 + g) * _SPG, _SPG, j, means[g], accs[g]) for g in range(2))
                return accs

            accs = lax.fori_loop(j_start, nb, body, zeros(2 if with_var else 0))
            if with_var:
                put_rstd(2 * var_pair, accs[0])
                put_rstd(2 * var_pair + 1, accs[1])

        def write_loop1(o, c):
            _branch(jnp.logical_and(o >= 1, o <= n_pairs - 2),
                    lambda: write_window(o, o * _W1, _W1, o + 1, 0),
                    lambda: write_window(o, o * _W1, _W1, None, jnp.where(o == 0, _DW, 0)))
            return c

        lax.fori_loop(0, n1, write_loop1, 0)

        def write_loop2(i, c):
            write_window(n1 + i, n1 * _W1 + i * _W2, _W2, None, 0, i == 0)
            return c

        lax.fori_loop(0, n2, write_loop2, 0)

        n_slabs = n * _SPU
        n_chunks = (n1 + n2) * nb
        for i in range(_DW):
            _branch(n2 > 0,
                    lambda: wr_wait(bs, n_slabs - _W2, _W2, nb - _DW + i, n_chunks - _DW + i),
                    lambda: wr_wait(bs, n_slabs - _W1, _W1, nb - _DW + i, n_chunks - _DW + i))
            if i == _DW - 1 - _W2R:
                @pl.when(r < n_rounds - 1)
                def _():
                    start_round_reads(bs + n_full * _SPU)
        return carry

    lax.fori_loop(0, n_rounds, round_body, 0)


def _compiler_params():
    base = dict(vmem_limit_bytes=110 * 1024 * 1024, disable_bounds_checks=True)
    try:
        return pltpu.CompilerParams(disable_semaphore_checks=True, **base)
    except TypeError:
        return pltpu.CompilerParams(**base)


@jax.jit
def pallas_standalone__groupnorm__prompt_kernel(x: jax.Array, g: jax.Array, b: jax.Array):
    B, C, H, W = x.shape
    cps = C // _G // _SPG
    n_slabs = B * _G * _SPG
    rgs = cps * H // 8
    wt = W // 128
    tps = rgs * wt
    n_units = B * _G // _GPU
    n_full = _UNITS_PER_ROUND
    n_rounds = -(-n_units // n_full)
    n_last = n_units - (n_rounds - 1) * n_full
    nb = tps // _BT
    assert C == 8 * 128 and H % 8 == 0 and W % 128 == 0 and nb % cps == 0 and _DW <= nb - 1 - _DR
    assert n_last >= 3 and sum(_PARTS) == _SPU and len(_PARTS) * _DR <= _NRSEM and _DW <= _NWSEM
    for nn in (n_full, n_last):
        assert nn * _GPU // 2 - 2 < _split_windows(nn * _SPU)[0]

    xl = x.reshape(n_slabs * rgs, 8, wt, 128).transpose(0, 2, 1, 3).reshape(n_slabs, tps, 8, 128)
    out = pl.pallas_call(
        functools.partial(_gn_kernel, n_rounds=n_rounds, n_full=n_full, n_last=n_last, tps=tps, cps=cps),
        in_specs=[pl.BlockSpec(memory_space=pl.ANY)] * 3,
        out_specs=pl.BlockSpec(memory_space=pl.ANY),
        out_shape=jax.ShapeDtypeStruct(xl.shape, x.dtype),
        scratch_shapes=[
            pltpu.VMEM((n_full * _SPU, tps, 8, 128), x.dtype),
            pltpu.VMEM((2, 8, 128), g.dtype),
            pltpu.VMEM((16, 128), jnp.float32),
            pltpu.SMEM((16, 128), jnp.float32),
            pltpu.SMEM((2 * _GPU * n_full,), jnp.float32),
            pltpu.SemaphoreType.DMA((_NRSEM,)),
            pltpu.SemaphoreType.DMA((_NWSEM,)),
            pltpu.SemaphoreType.DMA((3,)),
        ],
        compiler_params=_compiler_params(),
    )(xl, g.reshape(8, 128), b.reshape(8, 128))
    return out.reshape(n_slabs * rgs, wt, 8, 128).transpose(0, 2, 1, 3).reshape(B, C, H, W)
```
